```python
import os as _os
_os.environ.setdefault('JAX_PLATFORMS', 'cpu')
import jax
import jax.numpy as jnp

def _softmax(x, axis=-1):
    return jax.nn.softmax(x, axis=axis)

def _gelu(x):
    return jax.nn.gelu(x, approximate=True)

def _silu(x):
    return jax.nn.silu(x)

def _sigmoid(x):
    return jax.nn.sigmoid(x)

def _layernorm(x, axis=-1, eps=1e-05):
    m = jnp.mean(x, axis=axis, keepdims=True)
    v = jnp.var(x, axis=axis, keepdims=True)
    return (x - m) / jnp.sqrt(v + eps)

def _scatter_add(tgt, idx, src, axis=0):
    return tgt.at[idx].add(src)

def _segment_sum(src, seg, n):
    return jax.ops.segment_sum(src, seg, n)

class _Rng:

    def __init__(self, key):
        self._k = key

    def _next(self):
        self._k, sub = jax.random.split(self._k)
        return sub

    def normal(self, shape):
        return jax.random.normal(self._next(), shape, dtype=jnp.bfloat16)

    def randint(self, lo, hi, shape):
        return jax.random.randint(self._next(), shape, lo, hi, dtype=jnp.int32)

    def uniform(self, shape, lo=0.0, hi=1.0):
        return jax.random.uniform(self._next(), shape, jnp.bfloat16, lo, hi)

    def permutation(self, n):
        return jax.random.permutation(self._next(), n)
kernel_name = 'adaLN_cond__linear_attn_block__swiglu_ffn__prompt'

def setup_inputs():
    _rng = _Rng(jax.random.key(int.from_bytes(__import__("os").urandom(4), "little")))
    _w = lambda a: (lambda t: t.astype(jnp.bfloat16) if jnp.issubdtype(t.dtype, jnp.floating) else t)(jnp.asarray(a))

    def _A_setup():
        B, S, D = (1, 2048, 640)
        return {'x': _w((lambda *s: _rng.normal(s) * 0.05)(B, S, D)), 'wqkv': _w((lambda *s: _rng.normal(s) * 0.8)(D, 3 * D)), 'wo': _w((lambda *s: _rng.normal(s) * 0.05)(D, D))}
    _A_in = _A_setup()

    def _B_setup():
        B, S, D, F = (1, 2048, 640, 1728)
        return {'x': _w((lambda *s: _rng.normal(s) * 0.05)(B, S, D)), 'w_gate': _w((lambda *s: _rng.normal(s) * 0.05)(D, F)), 'w_up': _w((lambda *s: _rng.normal(s) * 0.05)(D, F)), 'w_down': _w((lambda *s: _rng.normal(s) * 0.05)(F, D))}
    _B_in = _B_setup()
    return {'A_x': _A_in['x'], 'A_wqkv': _A_in['wqkv'], 'A_wo': _A_in['wo'], 'B_x': _B_in['x'], 'B_w_gate': _B_in['w_gate'], 'B_w_up': _B_in['w_up'], 'B_w_down': _B_in['w_down'], 'c': _w((lambda *s: _rng.normal(s) * 0.05)(1, 640) * 8.0), 'w_mod': _w((lambda *s: _rng.normal(s) * 0.05)(640, 6 * 640) * 640 ** (-0.5) * 8.0)}

def reference(A_x, A_wqkv, A_wo, B_x, B_w_gate, B_w_up, B_w_down, c, w_mod):

    def _A_ref(x, wqkv, wo):
        B, S, D = x.shape
        H = 32
        Dh = D // H
        qkv = (lambda x, *d: x.transpose(*d))((x @ wqkv).reshape(B, S, 3, H, Dh), 2, 0, 3, 1, 4)
        q, k, v = (qkv[0], qkv[1], qkv[2])
        phi = lambda t: jnp.where(t > 0, t + 1, jnp.exp(t)) + 1e-06
        pq, pk = (phi(q), phi(k))
        kv = jnp.einsum('bhsd,bhse->bhde', pk, v)
        z = jnp.einsum('bhsd->bhd', pk)
        num = jnp.einsum('bhqd,bhde->bhqe', pq, kv)
        den = jnp.einsum('bhqd,bhd->bhq', pq, z)[..., None] + 1e-06
        o = num / den
        return (lambda x, *d: x.transpose(*d))(o, 0, 2, 1, 3).reshape(B, S, D) @ wo

    def _B_ref(x, w_gate, w_up, w_down):
        g = _silu(x @ w_gate)
        u = x @ w_up
        return g * u @ w_down
    x = A_x
    mod = (_silu(c) @ w_mod).reshape(c.shape[0], 6, 1, -1)
    sa, ca, ga, sb, cb, gb = (mod[:, 0].copy(), mod[:, 1].copy(), mod[:, 2].copy(), mod[:, 3].copy(), mod[:, 4].copy(), mod[:, 5].copy())
    h = _layernorm(x, axis=-1) * (1 + ca) + sa
    x = x + ga * _A_ref(h, A_wqkv, A_wo)
    h = _layernorm(x, axis=-1) * (1 + cb) + sb
    x = x + gb * _B_ref(h, B_w_gate, B_w_up, B_w_down)
    return x
```

```python
import jax
import jax.numpy as jnp
from jax import lax
import jax.experimental.pallas as pl
import jax.experimental.pallas.tpu as pltpu

S, D, F, H, DH = 2048, 640, 1728, 32, 20
T = 512
R = D // 4
NC = 6
FM = NC * 256
HL = (F - FM) // 2
RS, WS = 32, 16
f32, bf16 = jnp.float32, jnp.bfloat16
KV_ROWS = ((0, 144), (112, 272), (240, 400), (368, 528), (496, 640))
AS_RHS = (0, 2, 6, 5, 3, 4, 1)

PROGRAM = """
s:k,x0,c,ma w:k wk w:x0,c,ma s:xr,q mod K0 w:xr,q s:v,o,mb,g,u,d K1 K2 G01 K3 Q0 G23 w:v,o,mb,g,u,d
Q1/0/2 kv Q1/1/2 Q2/0/2 M Q2/1/2
A0 Q3 C00 C01 A1 C02 C10 C11 C03 C12 C04 C13 C05 C14 C06 C15 A2 C16 E0 D0 C20 C21 Y0 o0 E1 A3 D1
C30 C22 Y1 o1 C31 C23 C24 C25 C26 C36 E2 D2 C32 C33 Y2 o2 C34 C35 E3 D3 Y3
"""


def _quads(G):
    n = len(G) // 2
    return [r[:n] for r in G[:n]], [r[n:] for r in G[:n]], [r[:n] for r in G[n:]], [r[n:] for r in G[n:]]


def _add(P, Q): return [[a + b for a, b in zip(p, q)] for p, q in zip(P, Q)]
def _sub(P, Q): return [[a - b for a, b in zip(p, q)] for p, q in zip(P, Q)]


def lhs_terms(G, depth):
    if depth == 0:
        return [G]
    a11, a12, a21, a22 = _quads(G)
    return [t for g in (_add(a11, a22), _add(a21, a22), a11, a22, _add(a11, a12), _sub(a21, a11), _sub(a12, a22))
            for t in lhs_terms(g, depth - 1)]


def rhs_terms(G, depth):
    if depth == 0:
        return [G]
    b11, b12, b21, b22 = _quads(G)
    return [t for g in (_add(b11, b22), b11, _sub(b12, b22), _sub(b21, b11), b22, _add(b11, b12), _add(b21, b22))
            for t in rhs_terms(g, depth - 1)]


def out_blocks(M, extra=None):
    if len(M) == 1:
        return M[0]
    n = len(M) // 7
    m = [out_blocks(M[i * n:(i + 1) * n]) for i in range(7)]
    if extra is not None:
        m = [_add(a, b) for a, b in zip(m, extra)]
    c11 = _add(_sub(_add(m[0], m[3]), m[4]), m[6])
    c22 = _add(_add(_sub(m[0], m[1]), m[2]), m[5])
    return [a + b for a, b in zip(c11, _add(m[2], m[4]))] + [a + b for a, b in zip(_add(m[1], m[3]), c22)]


def staggered(depth):
    halves = ((0, 1), (1,), (0,), (1,), (0,), (0, 1), (0, 1))
    n = 7 ** depth

    def last_row(p):
        if p >= n:
            return p - n
        if depth == 1:
            return 2 * max(halves[p]) + 1
        return max(2 * i + j for i in halves[p // 7] for j in halves[p % 7])
    return sorted(range(n + 4), key=lambda p: (last_row(p), p < n))


def turn(G): return [list(r) for r in zip(*G)]
def flat(G): return [c for row in G for c in row]
def dot(a, b): return jnp.dot(a, b, preferred_element_type=f32)
def dot_nt(a, b): return lax.dot_general(a, b, (((1,), (1,)), ((), ())), preferred_element_type=f32)
def cat0(xs): return xs[0] if len(xs) == 1 else jnp.concatenate(xs, axis=0)
def cat1(xs): return xs[0] if len(xs) == 1 else jnp.concatenate(xs, axis=1)
def tiles(x): return [x[:, k * 128:(k + 1) * 128] for k in range(x.shape[1] // 128)]
def phi(t): return jnp.where(t > 0, t + (1.0 + 1e-6), jnp.exp(t) + 1e-6)
def silu(t): return t * pl.reciprocal(1.0 + jnp.exp(-t), approx=True)


def total(xs):
    s = xs[0]
    for x in xs[1:]:
        s = s + x
    return s


def norm_rows(x):
    mu = jnp.sum(total(tiles(x)), axis=1, keepdims=True) * (1.0 / D)
    xc = x - mu
    var = jnp.sum(total(tiles(xc * xc)), axis=1, keepdims=True) * (1.0 / D)
    return xc * lax.rsqrt(var + 1e-5)


def make_kernel(program):
    waits = [st[2:].split(',') for st in program if st[:2] == 'w:']

    def kernel(x_hbm, wqkv_hbm, wo_hbm, wg_hbm, wu_hbm, wd_hbm, c_hbm, wm_hbm, o_hbm,
               x_v, wq_v, wk_v, wv_v, wo_v, wg_v, wu_v, wd_v, c_v, wm_v, tq_v, tm_v, z_v, o_v, sem):
        src = {'c': (c_hbm, c_v), 'o': (wo_hbm, wo_v), 'g': (wg_hbm, wg_v), 'u': (wu_hbm, wu_v), 'd': (wd_hbm, wd_v)}
        for i, (n, ref) in enumerate((('q', wq_v), ('k', wk_v), ('v', wv_v))):
            src[n] = (wqkv_hbm.at[:, pl.ds(i * D, D)], ref)
        for n, cols in (('ma', pl.ds(0, 2 * D)), ('mb', pl.ds(2 * D, 4 * D))):
            src[n] = (wm_hbm.at[:, cols], wm_v.at[:, cols])
        for n, rows in (('x0', pl.ds(0, T)), ('xr', pl.ds(T, S - T))):
            src[n] = (x_hbm.at[rows], x_v.at[rows])
        d_in = {n: pltpu.make_async_copy(*src[n], sem.at[i]) for i, group in enumerate(waits) for n in group}
        v, cache, sent = {}, {}, []

        def alloc(depth):
            n = 4 >> depth
            return ([[[{} for _ in range(n)] for _ in range(n)] for _ in range(7 ** depth if depth else 0)],
                    [[{} for _ in range(1 if depth else 5)] for _ in range(4)])

        def put(L, r, terms):
            for l, t in zip(L, terms):
                for a, b in zip(flat(l), flat(t)):
                    a[r] = b

        def put_rows(op, r, rows, terms):
            put(op[0], r, terms([e[:4] for e in rows]))
            put([op[1]], r, [[e[4 if op[0] else 0:] for e in rows]])

        def get(grid):
            key = tuple(id(l) for l in flat(grid))
            if key not in cache:
                cache[key] = cat0([cat1([cat0([l[i] for i in sorted(l)]) for l in row]) for row in grid]).astype(bf16)
            return cache[key]

        def need(name, *a):
            if (name, *a) not in v:
                v[(name, *a)] = make[name](*a)
            return v[(name, *a)]

        def weight_terms(depth, rows, nr=R):
            op = alloc(depth)
            for r in range(0, nr, WS):
                put_rows(op, r, [rows(n, r) for n in range(4)], lambda W: [turn(t) for t in rhs_terms(turn(W), depth)])
            return op

        def products(key, depth, prod, plain, stagger):
            n = 7 ** depth if depth else 0
            M, rem = v[key] = [None] * n, [None] * 4

            def one(p):
                if p < n:
                    M[p] = prod(p)
                else:
                    rem[p - n] = plain(p - n)
            return one, staggered(depth) if stagger else list(range(n + 4))

        def project(key, depth, w, x, mul, stagger):
            return products(key, depth, lambda p: mul(w[0][p], x[0][p]), lambda a: mul(w[1], [x[1][a]]), stagger)

        def mul_nt(w, x): return dot_nt(get(w), get(x))
        def mul_nn(w, xt): return dot(get(w), get(turn(xt)))

        def split(m, r, nr, rs):
            return [[m[n * nr + r:n * nr + r + rs, a * 128:(a + 1) * 128] for n in range(m.shape[0] // nr)]
                    for a in range(m.shape[1] // 128)]

        def blocks(prod, r, nr):
            M, rem = prod
            if not M:
                return [[rem[a][n * nr + r:n * nr + r + RS] for n in range(4)] for a in range(4)]
            C = out_blocks([split(m, r, nr, RS) for m in M])
            return [[C[a][n] + rem[a][n * nr + r:n * nr + r + RS] for n in range(4)] for a in range(4)]

        def start_mod():
            s = c_v[...].astype(f32)
            v['s'] = jnp.broadcast_to(s / (1.0 + jnp.exp(-s)), (128, D)).T

        def mod(i):
            ref = wm_v.at[:, pl.ds(i * D, D)]
            return jnp.sum(total([ref[r:r + 16, :].astype(f32) * cat1([v['s'][r:r + 16]] * 5) for r in range(0, D, 16)]),
                           axis=0, keepdims=True)

        def x_rows(b, a, r): return x_v[pl.ds(b * T + a * 128 + r, RS), :].astype(f32)

        def wk():
            wt = [wk_v[k * 128:(k + 1) * 128, :].astype(f32).T for k in range(5)]
            return weight_terms(1, lambda n, r: [wt[k][n * R + r:n * R + r + WS] for k in range(5)])

        def cast_wk():
            for l in need('wk')[0] + [need('wk')[1]]:
                get(l)

        def wq():
            for k in range(5):
                tq_v[k] = wq_v[k * 128:(k + 1) * 128, :].astype(f32).T
            return weight_terms(1, lambda n, r: [tq_v[k, pl.ds(r % 32 * DH + 5 * n + r // 32, WS, stride=DH), :] for k in range(5)])

        def h1(b):
            xn = {(a, r): norm_rows(x_rows(b, a, r)) for a in range(4) for r in range(0, 128, RS)}
            scale = 1.0 + need('mod', 1)
            h = {k: tiles(t * scale + need('mod', 0)) for k, t in xn.items()}
            op = alloc(1)
            for r in range(0, 128, RS):
                put_rows(op, r, [h[a, r] for a in range(4)], lambda X: lhs_terms(X, 1))
            return op

        def K(b): return project(('K', b), 1, need('wk'), need('h1', b), mul_nt, True)
        def Q(b): return project(('Q', b), 1, need('wq'), need('h1', b), mul_nt, False)

        def pk(b):
            L, plain = alloc(1)[0], [[{} for _ in range(4)] for _ in range(4)]
            for r in range(0, R, RS):
                P = turn([[phi(c) for c in row] for row in blocks(v['K', b], r, R)])
                for n in range(4):
                    rows = pl.ds(n * R + r, RS)
                    z_v[rows, :] = total(P[n]) if b == 0 else z_v[rows, :] + total(P[n])
                put([plain], r, [P])
                put(L, r, lhs_terms(P, 1))
            return L, plain

        def G(*bs):
            old = v.get('G')
            ks = [need('pk', b) for b in bs]

            def prod(p):
                m = dot(cat1([get(k[0][p]) for k in ks]), cat0([get(v['h1', b][0][AS_RHS[p]]) for b in bs]))
                return m if old is None else old[0][p] + m

            def plain(n):
                m = dot(cat1([get([k[1][n]]) for k in ks]), cat0([get(v['h1', b][1]) for b in bs]))
                return m if old is None else old[1][n] + m
            return products('G', 1, prod, plain, True)

        def kv():
            M, rem = v['G']
            C = out_blocks([turn(split(m, 0, R, R)) for m in M])
            g = cat0([cat1(C[n] + [rem[n]]) for n in range(4)])
            v['kv'] = []
            for t, (r0, r1) in enumerate(KV_ROWS):
                part = dot(g[r0:r1].astype(bf16), wv_v[:, t * 128:(t + 1) * 128])
                col = lax.broadcasted_iota(jnp.int32, (1, 128), 1) + t * 128
                lo = jnp.floor((col.astype(f32) + 0.5) * (1.0 / DH)).astype(jnp.int32) * DH
                row = lax.broadcasted_iota(jnp.int32, part.shape, 0) + r0
                v['kv'].append(jnp.where((row >= lo) & (row < lo + DH), part, 0.0))

        def kv_wo():
            mm = [dot(part.astype(bf16), wo_v[t * 128:(t + 1) * 128, :]) for t, part in enumerate(v['kv'])]
            cuts = sorted(flat(KV_ROWS))
            for a0, a1 in zip(cuts[:-1], cuts[1:]):
                piece = total([mm[t][a0 - r0:a1 - r0] for t, (r0, r1) in enumerate(KV_ROWS) if r0 <= a0 and a1 <= r1]) * need('mod', 2)
                for n in range(5):
                    tm_v[n, a0:a1, :] = piece[:, n * 128:(n + 1) * 128]

        def wm():
            mt = [cat0([cat1([tm_v[e, pl.ds(5 * n + j, H, stride=DH), :] for e in range(5)]) for n in range(4)]).T for j in range(5)]
            return weight_terms(0, lambda n, r: [mt[k][n * R + r:n * R + r + WS] for k in range(5)])

        def z():
            return [jnp.broadcast_to(jnp.sum(z_v[pl.ds(j, H, stride=DH), :], axis=1, keepdims=True), (H, 128)) for j in range(DH)]

        def pq(b):
            op, zs = alloc(0), need('z')
            P = [[[phi(c) for c in row] for row in blocks(v['Q', b], H * j, R)] for j in range(5)]
            inv = [1.0 / (total([P[j][a][n] * zs[5 * n + j] for j in range(5) for n in range(4)]) + 1e-6) for a in range(4)]
            for n in range(4):
                put_rows(op, H * n, [[P[j][a][n] * inv[a] for j in range(5)] for a in range(4)], lambda X: [])
            return op

        def A(b): return project(('A', b), 0, need('wm'), need('pq', b), mul_nn, False)

        def untranspose(f):
            Y = [f(r) for r in range(0, R, RS)]
            return [cat0([C[a][n] for n in range(4) for C in Y]).T for a in range(4)]

        def h2(b):
            attn = untranspose(lambda r: blocks(v['A', b], r, R))
            shift, scale = need('mod', 3), 1.0 + need('mod', 4)
            op = alloc(2)
            x1 = v['x1', b] = [[] for _ in range(4)]
            for r in range(0, 128, RS):
                for a in range(4):
                    x1[a].append(x_rows(b, a, r) + attn[a][r:r + RS])
                put_rows(op, r, [tiles(norm_rows(x1[a][-1]) * scale + shift) for a in range(4)], lambda X: lhs_terms(X, 2))
            return op

        def wgu(c):
            def rows(n, r):
                if c < NC:
                    f0 = 512 * (c // 2) + 64 * (c % 2) + 128 * (2 * (n // 2) + r // 64) + r % 64
                else:
                    f0 = FM + HL * (n // 2) + r
                return tiles((wu_v if n % 2 else wg_v)[f0:f0 + WS, :].astype(f32))
            return weight_terms(2, rows, 128 if c < NC else HL)

        def wd(c):
            if c < NC // 2:
                wt = [wd_v[512 * c + 128 * k:512 * c + 128 * (k + 1), :].astype(f32).T for k in range(4)]
            else:
                wt = [cat0([wd_v[FM + HL * k:FM + HL * (k + 1), :].astype(f32), jnp.zeros((128 - HL, D), f32)]).T for k in range(2)]
            nr, depth = D // len(wt), len(wt) // 2
            L = [[[{}]] for _ in range(7 ** depth)]
            for r in range(0, nr, WS):
                put(L, r, rhs_terms([[w[n * nr + r:n * nr + r + WS] for n in range(len(wt))] for w in wt], depth))
            return L

        def C(b, c):
            first = ('h2', b) not in v
            return project(('C', b, c), 2, need('wgu', c), need('h2', b), mul_nt, first)

        def act(b, c):
            L = [[[{}]] for _ in range(49 if c < NC else 7)]
            if c < NC:
                for r in range(0, 64, RS):
                    B = [blocks(v['C', b, c], r + 64 * half, 128) for half in range(2)]
                    put(L, r, lhs_terms([[silu(B[k % 2][a][k // 2 * 2]) * B[k % 2][a][k // 2 * 2 + 1] for k in range(4)] for a in range(4)], 2))
            else:
                for r in range(0, HL, RS):
                    B = blocks(v['C', b, c], r, HL)
                    g = [[silu(B[a][2 * k]) * B[a][2 * k + 1] for k in range(2)] for a in range(4)]
                    put(L, r, lhs_terms([[cat1([g[2 * a][k], g[2 * a + 1][k]]) for k in range(2)] for a in range(2)], 1))
                put(L, HL, [[[jnp.zeros((128 - HL, 256), f32)]]] * 7)
            return L

        def E(b):
            w, g = need('wd', NC // 2), need('act', b, NC)
            v['E', b] = [dot(get(w[p]), get(g[p])) for p in range(7)]

        def down(b):
            w, g = [need('wd', c) for c in range(NC // 2)], [need('act', b, c) for c in range(NC)]
            M = v['D', b] = [None] * 49

            def one(p):
                M[p] = dot(get([[t[p][0][0] for t in w]]), get([t[p][0] for t in g]))
            return one, [p for p in staggered(2) if p < 49]

        def send(row, n):
            sent.append(pltpu.make_async_copy(o_v.at[pl.ds(row, n)], o_hbm.at[pl.ds(row, n)], sem.at[len(waits)]))
            sent[-1].start()

        def Y(b):
            y = untranspose(lambda r: out_blocks([[[m[r:r + RS]]] for m in v['D', b]], [split(e, r, R, RS) for e in v['E', b]]))
            for a in range(4):
                o_v[pl.ds(b * T + a * 128, 128), :] = (cat0(v['x1', b][a]) + need('mod', 5) * y[a]).astype(bf16)
                if (b + 1) * T == S:
                    send(b * T + a * 128, 128)

        make = dict(mod=mod, wk=wk, wq=wq, h1=h1, pk=pk, z=z, pq=pq, wm=wm, h2=h2, wgu=wgu, wd=wd, act=act)
        steps = dict(wk=cast_wk, mod=start_mod, K=K, Q=Q, G=G, kv=kv, M=kv_wo, A=A, C=C, E=E,
                     D=down, Y=Y, o=lambda b: send(b * T, T))
        begun = {}
        for step in program:
            if step[1:2] == ':':
                for n in step[2:].split(','):
                    d_in[n].start() if step[0] == 's' else d_in[n].wait()
                continue
            key, *part = step.split('/')
            name = key.rstrip('0123456789')
            if key not in begun:
                begun[key] = steps[name](*map(int, key[len(name):]))
            if begun[key]:
                one, order = begun[key]
                i, n = map(int, part or (0, 1))
                for p in order[len(order) * i // n:len(order) * (i + 1) // n]:
                    one(p)
        for d in sent:
            d.wait()

    return kernel, len(waits) + 1


def block(A_x, A_wqkv, A_wo, B_w_gate, B_w_up, B_w_down, c, w_mod, program=PROGRAM):
    kernel, num_sems = make_kernel(program.split())
    V, hbm = pltpu.VMEM, pl.BlockSpec(memory_space=pltpu.HBM)
    out = pl.pallas_call(
        kernel,
        in_specs=[hbm] * 8,
        out_specs=hbm,
        out_shape=jax.ShapeDtypeStruct((S, D), bf16),
        scratch_shapes=[V((S, D), bf16), V((D, D), bf16), V((D, D), bf16), V((D, D), bf16), V((D, D), bf16),
                        V((F, D), bf16), V((F, D), bf16), V((F, D), bf16), V((1, D), bf16), V((D, 6 * D), bf16),
                        V((5, D, 128), f32), V((5, D, 128), f32), V((D, 128), f32), V((S, D), bf16),
                        pltpu.SemaphoreType.DMA((num_sems,))],
        compiler_params=pltpu.CompilerParams(vmem_limit_bytes=120 * 1024 * 1024),
    )(A_x.reshape(S, D), A_wqkv, A_wo, B_w_gate.T, B_w_up.T, B_w_down, c, w_mod)
    return out.reshape(1, S, D)


@jax.jit
def pallas_adaLN_cond__linear_attn_block__swiglu_ffn__prompt_kernel(
    A_x: jax.Array,
    A_wqkv: jax.Array,
    A_wo: jax.Array,
    B_x: jax.Array,
    B_w_gate: jax.Array,
    B_w_up: jax.Array,
    B_w_down: jax.Array,
    c: jax.Array,
    w_mod: jax.Array,
):
    del B_x
    return block(A_x, A_wqkv, A_wo, B_w_gate, B_w_up, B_w_down, c, w_mod)
```

```python
import jax
import jax.numpy as jnp
from jax import lax
import jax.experimental.pallas as pl
import jax.experimental.pallas.tpu as pltpu

S, D, F, H, DH = 2048, 640, 1728, 32, 20
T = 512
R = D // 4
NC = 6
FM = NC * 256
HL = (F - FM) // 2
RS, WS = 32, 16
f32, bf16 = jnp.float32, jnp.bfloat16
KV_ROWS = ((0, 144), (112, 272), (240, 400), (368, 528), (496, 640))
AS_RHS = (0, 2, 6, 5, 3, 4, 1)

PROGRAM = """
s:k,x0,c,ma w:k,x0,c s:xr,q wk xn0 mod w:ma s:v,o,mb,g,u,d K0 w:xr,q K1 K2 G01 Q0 K3 G23 w:v,o,mb,g,u,d
kv Q1 Q2/0/2 M Q2/1/2 A0 Q3 C00 A1 C01 C10 C02 C11 A2 C03 C12 C20 C04 C21 C13 A3 C05 C22 C30 C14 C06 C31
C23 C15 C16 E0 C24 D0 C25 C26 Y0 D1 C32 o0 E1 C33 Y1 o1 C36 E2 D2 C34 Y2 C35 o2 D3 E3 Y3
"""


def _quads(G):
    n = len(G) // 2
    return [r[:n] for r in G[:n]], [r[n:] for r in G[:n]], [r[:n] for r in G[n:]], [r[n:] for r in G[n:]]


def _add(P, Q): return [[a + b for a, b in zip(p, q)] for p, q in zip(P, Q)]
def _sub(P, Q): return [[a - b for a, b in zip(p, q)] for p, q in zip(P, Q)]


def lhs_terms(G, depth):
    if depth == 0:
        return [G]
    a11, a12, a21, a22 = _quads(G)
    return [t for g in (_add(a11, a22), _add(a21, a22), a11, a22, _add(a11, a12), _sub(a21, a11), _sub(a12, a22))
            for t in lhs_terms(g, depth - 1)]


def rhs_terms(G, depth):
    if depth == 0:
        return [G]
    b11, b12, b21, b22 = _quads(G)
    return [t for g in (_add(b11, b22), b11, _sub(b12, b22), _sub(b21, b11), b22, _add(b11, b12), _add(b21, b22))
            for t in rhs_terms(g, depth - 1)]


def out_blocks(M, extra=None):
    if len(M) == 1:
        return M[0]
    n = len(M) // 7
    m = [out_blocks(M[i * n:(i + 1) * n]) for i in range(7)]
    if extra is not None:
        m = [_add(a, b) for a, b in zip(m, extra)]
    c11 = _add(_sub(_add(m[0], m[3]), m[4]), m[6])
    c22 = _add(_add(_sub(m[0], m[1]), m[2]), m[5])
    return [a + b for a, b in zip(c11, _add(m[2], m[4]))] + [a + b for a, b in zip(_add(m[1], m[3]), c22)]


def staggered(depth):
    halves = ((0, 1), (1,), (0,), (1,), (0,), (0, 1), (0, 1))
    n = 7 ** depth if depth else 0

    def last_row(p):
        if p >= n:
            return p - n
        if depth == 1:
            return 2 * max(halves[p]) + 1
        return max(2 * i + j for i in halves[p // 7] for j in halves[p % 7])
    return sorted(range(n + 4), key=lambda p: (last_row(p), p < n))


def turn(G): return [list(r) for r in zip(*G)]
def flat(G): return [c for row in G for c in row]
def dot(a, b): return jnp.dot(a, b, preferred_element_type=f32)
def dot_nt(a, b): return lax.dot_general(a, b, (((1,), (1,)), ((), ())), preferred_element_type=f32)
def cat0(xs): return xs[0] if len(xs) == 1 else jnp.concatenate(xs, axis=0)
def cat1(xs): return xs[0] if len(xs) == 1 else jnp.concatenate(xs, axis=1)
def tiles(x): return [x[:, k * 128:(k + 1) * 128] for k in range(x.shape[1] // 128)]
def phi(t): return jnp.where(t > 0, t + (1.0 + 1e-6), jnp.exp(t) + 1e-6)
def silu(t): return t * pl.reciprocal(1.0 + jnp.exp(-t), approx=True)


def total(xs):
    s = xs[0]
    for x in xs[1:]:
        s = s + x
    return s


def norm_rows(x):
    mu = jnp.sum(total(tiles(x)), axis=1, keepdims=True) * (1.0 / D)
    xc = x - mu
    var = jnp.sum(total(tiles(xc * xc)), axis=1, keepdims=True) * (1.0 / D)
    return xc * lax.rsqrt(var + 1e-5)


def make_kernel(program):
    waits = [st[2:].split(',') for st in program if st[:2] == 'w:']

    def kernel(x_hbm, wqkv_hbm, wo_hbm, wg_hbm, wu_hbm, wd_hbm, c_hbm, wm_hbm, o_hbm,
               x_v, wq_v, wk_v, wv_v, wo_v, wg_v, wu_v, wd_v, c_v, wm_v, tq_v, tm_v, z_v, o_v, sem):
        src = {'c': (c_hbm, c_v), 'o': (wo_hbm, wo_v), 'g': (wg_hbm, wg_v), 'u': (wu_hbm, wu_v), 'd': (wd_hbm, wd_v)}
        for i, (n, ref) in enumerate((('q', wq_v), ('k', wk_v), ('v', wv_v))):
            src[n] = (wqkv_hbm.at[:, pl.ds(i * D, D)], ref)
        for n, cols in (('ma', pl.ds(0, 2 * D)), ('mb', pl.ds(2 * D, 4 * D))):
            src[n] = (wm_hbm.at[:, cols], wm_v.at[:, cols])
        for n, rows in (('x0', pl.ds(0, T)), ('xr', pl.ds(T, S - T))):
            src[n] = (x_hbm.at[rows], x_v.at[rows])
        d_in = {n: pltpu.make_async_copy(*src[n], sem.at[i]) for i, group in enumerate(waits) for n in group}
        v, cache, sent = {}, {}, []

        def alloc(depth):
            n = 4 >> depth
            return ([[[{} for _ in range(n)] for _ in range(n)] for _ in range(7 ** depth if depth else 0)],
                    [[{} for _ in range(1 if depth else 5)] for _ in range(4)])

        def put(L, r, terms):
            for l, t in zip(L, terms):
                for a, b in zip(flat(l), flat(t)):
                    a[r] = b

        def put_rows(op, r, rows, terms):
            put(op[0], r, terms([e[:4] for e in rows]))
            put([op[1]], r, [[e[4 if op[0] else 0:] for e in rows]])

        def get(grid):
            key = tuple(id(l) for l in flat(grid))
            if key not in cache:
                cache[key] = cat0([cat1([cat0([l[i] for i in sorted(l)]) for l in row]) for row in grid]).astype(bf16)
            return cache[key]

        def need(name, *a):
            if (name, *a) not in v:
                v[(name, *a)] = make[name](*a)
            return v[(name, *a)]

        def weight_terms(depth, rows, nr=R):
            op = alloc(depth)
            for r in range(0, nr, WS):
                put_rows(op, r, [rows(n, r) for n in range(4)], lambda W: [turn(t) for t in rhs_terms(turn(W), depth)])
            return op

        def products(key, depth, prod, plain, stagger):
            n = 7 ** depth if depth else 0
            M, rem = v[key] = [None] * n, [None] * 4

            def one(p):
                if p < n:
                    M[p] = prod(p)
                else:
                    rem[p - n] = plain(p - n)
            orders = staggered(depth), list(range(n + 4))
            return one, orders if stagger else orders[::-1]

        def project(key, depth, w, x, mul, stagger):
            return products(key, depth, lambda p: mul(w[0][p], x[0][p]), lambda a: mul(w[1], [x[1][a]]), stagger)

        def mul_nt(w, x): return dot_nt(get(w), get(x))
        def mul_nn(w, xt): return dot(get(w), get(turn(xt)))

        def split(m, r, nr, rs):
            return [[m[n * nr + r:n * nr + r + rs, a * 128:(a + 1) * 128] for n in range(m.shape[0] // nr)]
                    for a in range(m.shape[1] // 128)]

        def blocks(prod, r, nr):
            M, rem = prod
            if not M:
                return [[rem[a][n * nr + r:n * nr + r + RS] for n in range(4)] for a in range(4)]
            C = out_blocks([split(m, r, nr, RS) for m in M])
            return [[C[a][n] + rem[a][n * nr + r:n * nr + r + RS] for n in range(4)] for a in range(4)]

        def start_mod():
            s = c_v[...].astype(f32)
            v['s'] = jnp.broadcast_to(s / (1.0 + jnp.exp(-s)), (128, D)).T

        def mod(i):
            ref = wm_v.at[:, pl.ds(i * D, D)]
            return jnp.sum(total([ref[r:r + 16, :].astype(f32) * cat1([v['s'][r:r + 16]] * 5) for r in range(0, D, 16)]),
                           axis=0, keepdims=True)

        def x_rows(b, a, r): return x_v[pl.ds(b * T + a * 128 + r, RS), :].astype(f32)

        def wk():
            wt = [wk_v[k * 128:(k + 1) * 128, :].astype(f32).T for k in range(5)]
            return weight_terms(1, lambda n, r: [wt[k][n * R + r:n * R + r + WS] for k in range(5)])

        def cast_wk():
            for l in need('wk')[0] + [need('wk')[1]]:
                get(l)

        def wq():
            for k in range(5):
                tq_v[k] = wq_v[k * 128:(k + 1) * 128, :].astype(f32).T
            return weight_terms(1, lambda n, r: [tq_v[k, pl.ds(r % 32 * DH + 5 * n + r // 32, WS, stride=DH), :] for k in range(5)])

        def xn(b):
            return {(a, r): norm_rows(x_rows(b, a, r)) for a in range(4) for r in range(0, 128, RS)}

        def h1(b):
            rows, scale = need('xn', b), 1.0 + need('mod', 1)
            h = {k: tiles(t * scale + need('mod', 0)) for k, t in rows.items()}
            op = alloc(1)
            for r in range(0, 128, RS):
                put_rows(op, r, [h[a, r] for a in range(4)], lambda X: lhs_terms(X, 1))
            return op

        def K(b): return project(('K', b), 1, need('wk'), need('h1', b), mul_nt, True)
        def Q(b): return project(('Q', b), 1, need('wq'), need('h1', b), mul_nt, False)

        def pk(b):
            L, plain = alloc(1)[0], [[{} for _ in range(4)] for _ in range(4)]
            for r in range(0, R, RS):
                P = turn([[phi(c) for c in row] for row in blocks(v['K', b], r, R)])
                for n in range(4):
                    rows = pl.ds(n * R + r, RS)
                    z_v[rows, :] = total(P[n]) if b == 0 else z_v[rows, :] + total(P[n])
                put([plain], r, [P])
                put(L, r, lhs_terms(P, 1))
            return L, plain

        def G(*bs):
            old = v.get('G')
            ks = [need('pk', b) for b in bs]

            def prod(p):
                m = dot(cat1([get(k[0][p]) for k in ks]), cat0([get(v['h1', b][0][AS_RHS[p]]) for b in bs]))
                return m if old is None else old[0][p] + m

            def plain(n):
                m = dot(cat1([get([k[1][n]]) for k in ks]), cat0([get(v['h1', b][1]) for b in bs]))
                return m if old is None else old[1][n] + m
            return products('G', 1, prod, plain, True)

        def kv():
            M, rem = v['G']
            C = out_blocks([turn(split(m, 0, R, R)) for m in M])
            g = cat0([cat1(C[n] + [rem[n]]) for n in range(4)])
            v['kv'] = []
            for t, (r0, r1) in enumerate(KV_ROWS):
                part = dot(g[r0:r1].astype(bf16), wv_v[:, t * 128:(t + 1) * 128])
                col = lax.broadcasted_iota(jnp.int32, (1, 128), 1) + t * 128
                lo = jnp.floor((col.astype(f32) + 0.5) * (1.0 / DH)).astype(jnp.int32) * DH
                row = lax.broadcasted_iota(jnp.int32, part.shape, 0) + r0
                v['kv'].append(jnp.where((row >= lo) & (row < lo + DH), part, 0.0))

        def kv_wo():
            mm = [dot(part.astype(bf16), wo_v[t * 128:(t + 1) * 128, :]) for t, part in enumerate(v['kv'])]
            cuts = sorted(flat(KV_ROWS))
            for a0, a1 in zip(cuts[:-1], cuts[1:]):
                piece = total([mm[t][a0 - r0:a1 - r0] for t, (r0, r1) in enumerate(KV_ROWS) if r0 <= a0 and a1 <= r1]) * need('mod', 2)
                for n in range(5):
                    tm_v[n, a0:a1, :] = piece[:, n * 128:(n + 1) * 128]

        def wm():
            mt = [cat0([cat1([tm_v[e, pl.ds(5 * n + j, H, stride=DH), :] for e in range(5)]) for n in range(4)]).T for j in range(5)]
            return weight_terms(0, lambda n, r: [mt[k][n * R + r:n * R + r + WS] for k in range(5)])

        def z():
            return [jnp.broadcast_to(jnp.sum(z_v[pl.ds(j, H, stride=DH), :], axis=1, keepdims=True), (H, 128)) for j in range(DH)]

        def pq(b):
            op, zs = alloc(0), need('z')
            P = [[[phi(c) for c in row] for row in blocks(v['Q', b], H * j, R)] for j in range(5)]
            inv = [1.0 / (total([P[j][a][n] * zs[5 * n + j] for j in range(5) for n in range(4)]) + 1e-6) for a in range(4)]
            for n in range(4):
                put_rows(op, H * n, [[P[j][a][n] * inv[a] for j in range(5)] for a in range(4)], lambda X: [])
            return op

        def A(b): return project(('A', b), 0, need('wm'), need('pq', b), mul_nn, False)

        def untranspose(f):
            Y = [f(r) for r in range(0, R, RS)]
            return [cat0([C[a][n] for n in range(4) for C in Y]).T for a in range(4)]

        def h2(b):
            attn = untranspose(lambda r: blocks(v['A', b], r, R))
            shift, scale = need('mod', 3), 1.0 + need('mod', 4)
            op = alloc(2)
            x1 = v['x1', b] = [[] for _ in range(4)]
            for r in range(0, 128, RS):
                for a in range(4):
                    x1[a].append(x_rows(b, a, r) + attn[a][r:r + RS])
                put_rows(op, r, [tiles(norm_rows(x1[a][-1]) * scale + shift) for a in range(4)], lambda X: lhs_terms(X, 2))
            return op

        def wgu(c):
            def rows(n, r):
                if c < NC:
                    f0 = 512 * (c // 2) + 64 * (c % 2) + 128 * (2 * (n // 2) + r // 64) + r % 64
                else:
                    f0 = FM + HL * (n // 2) + r
                return tiles((wu_v if n % 2 else wg_v)[f0:f0 + WS, :].astype(f32))
            return weight_terms(2, rows, 128 if c < NC else HL)

        def wd(c):
            if c < NC // 2:
                wt = [wd_v[512 * c + 128 * k:512 * c + 128 * (k + 1), :].astype(f32).T for k in range(4)]
            else:
                wt = [cat0([wd_v[FM + HL * k:FM + HL * (k + 1), :].astype(f32), jnp.zeros((128 - HL, D), f32)]).T for k in range(2)]
            nr, depth = D // len(wt), len(wt) // 2
            L = [[[{}]] for _ in range(7 ** depth)]
            for r in range(0, nr, WS):
                put(L, r, rhs_terms([[w[n * nr + r:n * nr + r + WS] for n in range(len(wt))] for w in wt], depth))
            return L

        def C(b, c):
            first = ('h2', b) not in v
            return project(('C', b, c), 2, need('wgu', c), need('h2', b), mul_nt, first)

        def act(b, c):
            L = [[[{}]] for _ in range(49 if c < NC else 7)]
            if c < NC:
                for r in range(0, 64, RS):
                    B = [blocks(v['C', b, c], r + 64 * half, 128) for half in range(2)]
                    put(L, r, lhs_terms([[silu(B[k % 2][a][k // 2 * 2]) * B[k % 2][a][k // 2 * 2 + 1] for k in range(4)] for a in range(4)], 2))
            else:
                for r in range(0, HL, RS):
                    B = blocks(v['C', b, c], r, HL)
                    g = [[silu(B[a][2 * k]) * B[a][2 * k + 1] for k in range(2)] for a in range(4)]
                    put(L, r, lhs_terms([[cat1([g[2 * a][k], g[2 * a + 1][k]]) for k in range(2)] for a in range(2)], 1))
                put(L, HL, [[[jnp.zeros((128 - HL, 256), f32)]]] * 7)
            return L

        def E(b):
            w, g = need('wd', NC // 2), need('act', b, NC)
            v['E', b] = [dot(get(w[p]), get(g[p])) for p in range(7)]

        def down(b):
            w, g = [need('wd', c) for c in range(NC // 2)], [need('act', b, c) for c in range(NC)]
            M = v['D', b] = [None] * 49

            def one(p):
                M[p] = dot(get([[t[p][0][0] for t in w]]), get([t[p][0] for t in g]))
            return one, ([p for p in staggered(2) if p < 49], list(range(49)))

        def send(row, n):
            sent.append(pltpu.make_async_copy(o_v.at[pl.ds(row, n)], o_hbm.at[pl.ds(row, n)], sem.at[len(waits)]))
            sent[-1].start()

        def Y(b):
            y = untranspose(lambda r: out_blocks([[[m[r:r + RS]]] for m in v['D', b]], [split(e, r, R, RS) for e in v['E', b]]))
            for a in range(4):
                o_v[pl.ds(b * T + a * 128, 128), :] = (cat0(v['x1', b][a]) + need('mod', 5) * y[a]).astype(bf16)
                if (b + 1) * T == S:
                    send(b * T + a * 128, 128)

        make = dict(mod=mod, xn=xn, wk=wk, wq=wq, h1=h1, pk=pk, z=z, pq=pq, wm=wm, h2=h2, wgu=wgu, wd=wd, act=act)
        steps = dict(wk=cast_wk, mod=start_mod, xn=lambda b: need('xn', b) and None, K=K, Q=Q, G=G, kv=kv, M=kv_wo, A=A, C=C, E=E,
                     D=down, Y=Y, o=lambda b: send(b * T, T))
        begun = {}
        for step in program:
            if step[1:2] == ':':
                for n in step[2:].split(','):
                    d_in[n].start() if step[0] == 's' else d_in[n].wait()
                continue
            key, *part = step.rstrip('!').split('/')
            name = key.rstrip('0123456789')
            if key not in begun:
                begun[key] = steps[name](*map(int, key[len(name):]))
            if begun[key]:
                one, orders = begun[key]
                order = orders[step.endswith('!')]
                i, n = map(int, part or (0, 1))
                for p in order[len(order) * i // n:len(order) * (i + 1) // n]:
                    one(p)
        for d in sent:
            d.wait()

    return kernel, len(waits) + 1


def block(A_x, A_wqkv, A_wo, B_w_gate, B_w_up, B_w_down, c, w_mod, program=PROGRAM):
    kernel, num_sems = make_kernel(program.split())
    V, hbm = pltpu.VMEM, pl.BlockSpec(memory_space=pltpu.HBM)
    out = pl.pallas_call(
        kernel,
        in_specs=[hbm] * 8,
        out_specs=hbm,
        out_shape=jax.ShapeDtypeStruct((S, D), bf16),
        scratch_shapes=[V((S, D), bf16), V((D, D), bf16), V((D, D), bf16), V((D, D), bf16), V((D, D), bf16),
                        V((F, D), bf16), V((F, D), bf16), V((F, D), bf16), V((1, D), bf16), V((D, 6 * D), bf16),
                        V((5, D, 128), f32), V((5, D, 128), f32), V((D, 128), f32), V((S, D), bf16),
                        pltpu.SemaphoreType.DMA((num_sems,))],
        compiler_params=pltpu.CompilerParams(vmem_limit_bytes=126 * 1024 * 1024),
    )(A_x.reshape(S, D), A_wqkv, A_wo, B_w_gate.T, B_w_up.T, B_w_down, c, w_mod)
    return out.reshape(1, S, D)


@jax.jit
def pallas_adaLN_cond__linear_attn_block__swiglu_ffn__prompt_kernel(
    A_x: jax.Array,
    A_wqkv: jax.Array,
    A_wo: jax.Array,
    B_x: jax.Array,
    B_w_gate: jax.Array,
    B_w_up: jax.Array,
    B_w_down: jax.Array,
    c: jax.Array,
    w_mod: jax.Array,
):
    del B_x
    return block(A_x, A_wqkv, A_wo, B_w_gate, B_w_up, B_w_down, c, w_mod)
```
